```python
import os as _os
_os.environ.setdefault("JAX_PLATFORMS", "cpu")
import jax
import jax.numpy as jnp

def _softmax(x, axis=-1):
    return jax.nn.softmax(x, axis=axis)
def _gelu(x):
    return jax.nn.gelu(x, approximate=True)
def _silu(x):
    return jax.nn.silu(x)
def _sigmoid(x):
    return jax.nn.sigmoid(x)
def _layernorm(x, axis=-1, eps=1e-5):
    m = jnp.mean(x, axis=axis, keepdims=True)
    v = jnp.var(x, axis=axis, keepdims=True)
    return (x - m) / jnp.sqrt(v + eps)
def _scatter_add(tgt, idx, src, axis=0):
    return tgt.at[idx].add(src)
def _segment_sum(src, seg, n):
    return jax.ops.segment_sum(src, seg, n)
class _Rng:
    def __init__(self, key):
        self._k = key
    def _next(self):
        self._k, sub = jax.random.split(self._k)
        return sub
    def normal(self, shape):
        return jax.random.normal(self._next(), shape, dtype=jnp.bfloat16)
    def randint(self, lo, hi, shape):
        return jax.random.randint(self._next(), shape, lo, hi, dtype=jnp.int32)
    def uniform(self, shape, lo=0.0, hi=1.0):
        return jax.random.uniform(self._next(), shape, jnp.bfloat16, lo, hi)
    def permutation(self, n):
        return jax.random.permutation(self._next(), n)


kernel_name = 'standalone__mha_softmax__near_ridge'

def setup_inputs():
    _rng = _Rng(jax.random.key(int.from_bytes(__import__("os").urandom(4), "little")))
    _w = (lambda a: (lambda t: t.astype(jnp.bfloat16) if jnp.issubdtype(t.dtype, jnp.floating) else t)(jnp.asarray(a)))
    B, H, Sq, Sk, D = 16, 16, 256, 256, 256
    return {
        "q": _w((lambda *s: _rng.normal(s) * 0.4)(B, H, Sq, D)),
        "k": _w((lambda *s: _rng.normal(s) * 0.4)(B, H, Sk, D)),
        "v": _w((lambda *s: _rng.normal(s) * 0.05)(B, H, Sk, D)),
    }

def reference(q, k, v):
    scale = q.shape[-1] ** -0.5
    scores = jnp.einsum("bhqd,bhkd->bhqk", q, k) * scale
    p = _softmax(scores, axis=-1)
    return jnp.einsum("bhqk,bhkd->bhqd", p, v)
```

```python
import math

import jax
import jax.numpy as jnp
import jax.experimental.pallas as pl
import jax.experimental.pallas.tpu as pltpu

_LOG2E = math.log2(math.e)

_HEADS_PER_STEP = 8


def _attention_head(q, k, v, scale):
    s = jax.lax.dot_general(
        q, k, (((1,), (1,)), ((), ())), preferred_element_type=jnp.float32
    )
    m = jnp.max(s, axis=-1, keepdims=True)
    p = jnp.exp2((s - m) * (scale * _LOG2E))
    l = jnp.sum(p, axis=-1, keepdims=True)
    o = jnp.dot(p.astype(v.dtype), v, preferred_element_type=jnp.float32)
    return o * (1.0 / l)


@jax.jit
def pallas_standalone__mha_softmax__near_ridge_kernel(
    q: jax.Array,
    k: jax.Array,
    v: jax.Array,
):
    B, H, S, D = q.shape
    BH = B * H
    HB = _HEADS_PER_STEP
    assert BH % HB == 0
    scale = float(D) ** -0.5

    q3 = q.reshape(BH, S, D)
    k3 = k.reshape(BH, S, D)
    v3 = v.reshape(BH, S, D)

    def kernel_function(q_ref, k_ref, v_ref, o_ref):
        i = pl.program_id(0)
        for h in range(HB):
            o_ref[i * HB + h] = _attention_head(
                q_ref[h], k_ref[h], v_ref[h], scale
            ).astype(o_ref.dtype)

    in_spec = pl.BlockSpec((HB, S, D), lambda i: (i, 0, 0))
    out_spec = pl.BlockSpec(
        (BH, S, D), lambda i: (0, 0, 0), pipeline_mode=pl.Buffered(1)
    )

    out = pl.pallas_call(
        kernel_function,
        grid=(BH // HB,),
        in_specs=[in_spec, in_spec, in_spec],
        out_specs=out_spec,
        out_shape=jax.ShapeDtypeStruct((BH, S, D), q.dtype),
        compiler_params=pltpu.CompilerParams(
            dimension_semantics=("arbitrary",),
            vmem_limit_bytes=100 * 1024 * 1024,
        ),
    )(q3, k3, v3)
    return out.reshape(B, H, S, D)
```

```python
import math

import jax
import jax.numpy as jnp
import jax.experimental.pallas as pl
import jax.experimental.pallas.tpu as pltpu

_LOG2E = math.log2(math.e)

_HEADS_PER_STEP = 8


def _attention_head(q, k, v, scale):
    s = jax.lax.dot_general(
        q, k, (((1,), (1,)), ((), ())), preferred_element_type=jnp.float32
    )
    m = jnp.max(s, axis=-1, keepdims=True)
    p = jnp.exp2((s - m) * (scale * _LOG2E))
    l = jnp.sum(p, axis=-1, keepdims=True)
    o = jnp.dot(p.astype(v.dtype), v, preferred_element_type=jnp.float32)
    return o * (1.0 / l)


@jax.jit
def pallas_standalone__mha_softmax__near_ridge_kernel(
    q: jax.Array,
    k: jax.Array,
    v: jax.Array,
):
    B, H, S, D = q.shape
    BH = B * H
    HB = _HEADS_PER_STEP
    assert BH % HB == 0
    n_steps = BH // HB
    assert n_steps >= 2
    last = n_steps - 1
    scale = float(D) ** -0.5

    q3 = q.reshape(BH, S, D)
    k3 = k.reshape(BH, S, D)
    v3 = v.reshape(BH, S, D)

    def step_in_block(i):
        return jnp.where(i == last, 0, i)

    def kernel_function(q_ref, k_ref, v_ref, o_ref):
        base = step_in_block(pl.program_id(0)) * HB
        for h in range(HB):
            o_ref[base + h] = _attention_head(
                q_ref[h], k_ref[h], v_ref[h], scale
            ).astype(o_ref.dtype)

    in_spec = pl.BlockSpec((HB, S, D), lambda i: (i, 0, 0))
    out_spec = pl.BlockSpec(
        (BH - HB, S, D), lambda i: (jnp.where(i == last, 1, 0), 0, 0)
    )

    out = pl.pallas_call(
        kernel_function,
        grid=(n_steps,),
        in_specs=[in_spec, in_spec, in_spec],
        out_specs=out_spec,
        out_shape=jax.ShapeDtypeStruct((BH, S, D), q.dtype),
        compiler_params=pltpu.CompilerParams(
            dimension_semantics=("arbitrary",),
            vmem_limit_bytes=100 * 1024 * 1024,
        ),
    )(q3, k3, v3)
    return out.reshape(B, H, S, D)
```

```python
import math

import jax
import jax.numpy as jnp
import jax.experimental.pallas as pl
import jax.experimental.pallas.tpu as pltpu

_LOG2E = math.log2(math.e)

_HEADS_PER_STEP = 8


def _attention_head(q, k, v, scale):
    s = jax.lax.dot_general(
        q, k, (((1,), (1,)), ((), ())), preferred_element_type=jnp.float32
    )
    s = s.astype(q.dtype).astype(jnp.float32)
    if math.frexp(scale)[0] == 0.5:
        exp_scale = scale * _LOG2E
    else:
        s = (s * float(jnp.asarray(scale, q.dtype))).astype(q.dtype).astype(jnp.float32)
        exp_scale = _LOG2E
    m = jnp.max(s, axis=-1, keepdims=True)
    p = jnp.exp2((s - m) * exp_scale)
    l = jnp.sum(p, axis=-1, keepdims=True)
    o = jnp.dot(p.astype(v.dtype), v, preferred_element_type=jnp.float32)
    return o * (1.0 / l)


@jax.jit
def pallas_standalone__mha_softmax__near_ridge_kernel(
    q: jax.Array,
    k: jax.Array,
    v: jax.Array,
):
    B, H, S, D = q.shape
    BH = B * H
    HB = _HEADS_PER_STEP
    assert BH % HB == 0
    n_steps = BH // HB
    assert n_steps >= 2
    last = n_steps - 1
    scale = float(D) ** -0.5

    q3 = q.reshape(BH, S, D)
    k3 = k.reshape(BH, S, D)
    v3 = v.reshape(BH, S, D)

    def kernel_function(q_ref, k_ref, v_ref, o_ref):
        i = pl.program_id(0)
        base = jnp.where(i == last, 0, i) * HB
        for h in range(HB):
            o_ref[base + h] = _attention_head(
                q_ref[h], k_ref[h], v_ref[h], scale
            ).astype(o_ref.dtype)

    in_spec = pl.BlockSpec((HB, S, D), lambda i: (i, 0, 0))
    out_spec = pl.BlockSpec(
        (BH - HB, S, D), lambda i: (jnp.where(i == last, 1, 0), 0, 0)
    )

    out = pl.pallas_call(
        kernel_function,
        grid=(n_steps,),
        in_specs=[in_spec, in_spec, in_spec],
        out_specs=out_spec,
        out_shape=jax.ShapeDtypeStruct((BH, S, D), q.dtype),
        compiler_params=pltpu.CompilerParams(
            dimension_semantics=("arbitrary",),
            vmem_limit_bytes=100 * 1024 * 1024,
        ),
    )(q3, k3, v3)
    return out.reshape(B, H, S, D)
```

```python
import math

import jax
import jax.numpy as jnp
import jax.experimental.pallas as pl
import jax.experimental.pallas.tpu as pltpu

_LOG2E = math.log2(math.e)

_HEADS_PER_STEP = 8


def _round_to_bf16(x):
    m, e = math.frexp(x)
    return math.ldexp(round(m * 256.0), e - 8)


def _attention_head(q, k, v, scale):
    s = jax.lax.dot_general(
        q, k, (((1,), (1,)), ((), ())), preferred_element_type=jnp.float32
    )
    s = s.astype(q.dtype).astype(jnp.float32)
    if math.frexp(scale)[0] == 0.5:
        exp_scale = scale * _LOG2E
    else:
        s = (s * _round_to_bf16(scale)).astype(q.dtype).astype(jnp.float32)
        exp_scale = _LOG2E
    m = jnp.max(s, axis=-1, keepdims=True)
    p = jnp.exp2((s - m) * exp_scale)
    l = jnp.sum(p, axis=-1, keepdims=True)
    o = jnp.dot(p.astype(v.dtype), v, preferred_element_type=jnp.float32)
    return o * (1.0 / l)


@jax.jit
def pallas_standalone__mha_softmax__near_ridge_kernel(
    q: jax.Array,
    k: jax.Array,
    v: jax.Array,
):
    B, H, S, D = q.shape
    BH = B * H
    HB = _HEADS_PER_STEP
    assert BH % HB == 0
    n_steps = BH // HB
    assert n_steps >= 2
    last = n_steps - 1
    scale = float(D) ** -0.5

    q3 = q.reshape(BH, S, D)
    k3 = k.reshape(BH, S, D)
    v3 = v.reshape(BH, S, D)

    def kernel_function(q_ref, k_ref, v_ref, o_ref):
        i = pl.program_id(0)
        base = jnp.where(i == last, 0, i) * HB
        for h in range(HB):
            o_ref[base + h] = _attention_head(
                q_ref[h], k_ref[h], v_ref[h], scale
            ).astype(o_ref.dtype)

    in_spec = pl.BlockSpec((HB, S, D), lambda i: (i, 0, 0))
    out_spec = pl.BlockSpec(
        (BH - HB, S, D), lambda i: (jnp.where(i == last, 1, 0), 0, 0)
    )

    out = pl.pallas_call(
        kernel_function,
        grid=(n_steps,),
        in_specs=[in_spec, in_spec, in_spec],
        out_specs=out_spec,
        out_shape=jax.ShapeDtypeStruct((BH, S, D), q.dtype),
        compiler_params=pltpu.CompilerParams(
            dimension_semantics=("arbitrary",),
            vmem_limit_bytes=100 * 1024 * 1024,
        ),
    )(q3, k3, v3)
    return out.reshape(B, H, S, D)
```
